```python
import os as _os
_os.environ.setdefault("JAX_PLATFORMS", "cpu")
import jax
import jax.numpy as jnp

def _softmax(x, axis=-1):
    return jax.nn.softmax(x, axis=axis)
def _gelu(x):
    return jax.nn.gelu(x, approximate=True)
def _silu(x):
    return jax.nn.silu(x)
def _sigmoid(x):
    return jax.nn.sigmoid(x)
def _layernorm(x, axis=-1, eps=1e-5):
    m = jnp.mean(x, axis=axis, keepdims=True)
    v = jnp.var(x, axis=axis, keepdims=True)
    return (x - m) / jnp.sqrt(v + eps)
def _scatter_add(tgt, idx, src, axis=0):
    return tgt.at[idx].add(src)
def _segment_sum(src, seg, n):
    return jax.ops.segment_sum(src, seg, n)
class _Rng:
    def __init__(self, key):
        self._k = key
    def _next(self):
        self._k, sub = jax.random.split(self._k)
        return sub
    def normal(self, shape):
        return jax.random.normal(self._next(), shape, dtype=jnp.bfloat16)
    def randint(self, lo, hi, shape):
        return jax.random.randint(self._next(), shape, lo, hi, dtype=jnp.int32)
    def uniform(self, shape, lo=0.0, hi=1.0):
        return jax.random.uniform(self._next(), shape, jnp.bfloat16, lo, hi)
    def permutation(self, n):
        return jax.random.permutation(self._next(), n)


kernel_name = 'parallel_sum__linear_kernel_hedgehog__dense_activation_gelu__prompt'

def setup_inputs():
    _rng = _Rng(jax.random.key(int.from_bytes(__import__("os").urandom(4), "little")))
    _w = (lambda a: (lambda t: t.astype(jnp.bfloat16) if jnp.issubdtype(t.dtype, jnp.floating) else t)(jnp.asarray(a)))
    def _A_setup():
        B, S, D, H = 1, 2048, 448, 16
        Dh = D // H
        return {
            "x": _w((lambda *s: _rng.normal(s) * 0.05)(B, S, D)),
            "wqkv": _w((lambda *s: _rng.normal(s) * 0.2)(D, 3 * D)),
            "w_phi": _w((lambda *s: _rng.normal(s) * 0.2)(H, Dh, Dh) * (Dh ** -0.5)),
            "wo": _w((lambda *s: _rng.normal(s) * 0.05)(D, D)),
        }
    _A_in = _A_setup()

    def _B_setup():
        B, S, D, F = 1, 2048, 448, 1792
        return {
            "x": _w((lambda *s: _rng.normal(s) * 0.05)(B, S, D)),
            "w1": _w((lambda *s: _rng.normal(s) * 0.2)(D, F) * (D ** -0.5)),
            "b1": _w((lambda *s: _rng.normal(s) * 0.2)(F) * 0.01),
            "w2": _w((lambda *s: _rng.normal(s) * 0.2)(F, D) * (F ** -0.5)),
            "b2": _w((lambda *s: _rng.normal(s) * 0.05)(D) * 0.01),
        }
    _B_in = _B_setup()

    return {
        "A_x": _A_in["x"],
        "A_wqkv": _A_in["wqkv"],
        "A_w_phi": _A_in["w_phi"],
        "A_wo": _A_in["wo"],
        "B_x": _B_in["x"],
        "B_w1": _B_in["w1"],
        "B_b1": _B_in["b1"],
        "B_w2": _B_in["w2"],
        "B_b2": _B_in["b2"],
    }

def reference(A_x, A_wqkv, A_w_phi, A_wo, B_x, B_w1, B_b1, B_w2, B_b2):
    def _A_ref(x, wqkv, w_phi, wo):
        B, S, D = x.shape
        H = 16; Dh = D // H
        qkv = (lambda x, *d: x.transpose(*d))((x @ wqkv).reshape(B, S, 3, H, Dh), 2, 0, 3, 1, 4)
        q, k, v = qkv[0], qkv[1], qkv[2]
        pq = jnp.einsum("bhsd,hdf->bhsf", q, w_phi)
        pk = jnp.einsum("bhsd,hdf->bhsf", k, w_phi)
        phi_q = jnp.concatenate([_softmax(pq, axis=-1), _softmax(-pq, axis=-1)], axis=-1)
        phi_k = jnp.concatenate([_softmax(pk, axis=-1), _softmax(-pk, axis=-1)], axis=-1)
        kv = jnp.einsum("bhsf,bhsd->bhfd", phi_k, v)
        z  = jnp.einsum("bhsf->bhf", phi_k)
        num = jnp.einsum("bhqf,bhfd->bhqd", phi_q, kv)
        den = jnp.einsum("bhqf,bhf->bhq", phi_q, z)[..., None] + 1e-6
        o = num / den
        return (lambda x, *d: x.transpose(*d))(o, 0, 2, 1, 3).reshape(B, S, D) @ wo

    def _B_ref(x, w1, b1, w2, b2):
        h = jnp.einsum("bsd,df->bsf", x, w1) + b1
        h = _gelu(h)
        return jnp.einsum("bsf,fd->bsd", h, w2) + b2

    x = A_x
    xn = _layernorm(x, axis=-1)
    return x + _A_ref(xn, A_wqkv, A_w_phi, A_wo) + _B_ref(xn, B_w1, B_b1, B_w2, B_b2)
```

```python
import functools
import jax
import jax.numpy as jnp
from jax import lax
from jax.experimental import pallas as pl
from jax.experimental.pallas import tpu as pltpu

S, D, H, DH, F = 2048, 448, 16, 28, 1792
NT = (((1,), (1,)), ((), ()))
T = 512
NTL = S // T
FC = 256
NC = F // FC
LNC = 128
SEQ0 = "|x0 K00 K01 K02 K03 |wB,x1,wC v P0 P1 P2 P3 Q0 V00 Q1 V01 Q2 V02 Q3 V03 K10 V10 K11 V11 K12 K13 V12 |x2,x3,b1,b2,w1,w2,wo V13 K20 k00 k01 V20 k02 k03 K21 k04 k05 V21 k06 k07 K22 k10 k11 V22 k12 k13 K23 k14 k15 V23 k16 k17 a0 K30 V30 a1 K31 k20 k21 V31 k22 k23 b0 K32 k24 k25 V32 k26 k27 a2 K33 V33 b1 k30 k31 k32 k33 k34 k35 k36 k37 a3 b2 n0 n1 a4 b3 n2 n3 a5 b4 n4 n5 a6 b5 n6 n7 b6 w"
SEQN = "q0 q1 q2 q3 a0 a1 b0 n0 a2 n1 b1 n2 a3 n3 b2 n4 a4 n5 b3 n6 a5 n7 b4 a6 w b5 b6"
f32 = jnp.float32
LOG2E = 1.4426950408889634
GC = 0.7978845608028654
bf16 = jnp.bfloat16
P = functools.partial


def _iota(shape, dim):
    return lax.broadcasted_iota(jnp.int32, shape, dim)


def _divmod_const(i, n):
    q = jnp.floor((i.astype(f32) + 0.5) * (1.0 / n)).astype(jnp.int32)
    return q, i - q * n


def _fold(x, op):
    x = op(x, pltpu.roll(x, 4, 0))
    return op(x, pltpu.roll(x, 2, 0))


def _features(pg, t):
    p = pg.reshape(7, 8, t)
    mx = _fold(jnp.max(p, axis=0), jnp.maximum)
    mn = _fold(jnp.min(p, axis=0), jnp.minimum)

    def half(e):
        s = _fold(jnp.sum(e, axis=0), jnp.add)
        return (e * pl.reciprocal(s, approx=True)[None]).reshape(56, t)

    pos = half(jnp.exp2(p - mx[None]))
    neg = half(jnp.exp2(mn[None] - p))
    return jnp.concatenate([pos, neg], axis=0).astype(bf16)


def _kernel(x_hbm, wqkv_hbm, wphi_hbm, wo_hbm, w1_hbm, b1_hbm, w2T_hbm, b2_hbm, o_ref,
            x_s, wqkv_s, wphi_s, wo_s, w1_s, b1_s, w2T_s, b2_s, sems,
            xn_s, pq_s, pk0, pk1, pk2, pk3, va0, va1, va2, va3, wall_s, woT_s, w1T_s, kv_s, tmpa_s, tmpb_s, wfl_s):
    step = pl.program_id(0)
    pks = [pk0, pk1, pk2, pk3]
    vas = [va0, va1, va2, va3]

    class Tile:
        def __init__(self, cols, pre_f1=None, pre_wo=None):
            self.cols = cols
            self.h = {}
            self.acc = None
            self.os = []
            self.pre_f1 = pre_f1
            self.pre_wo = pre_wo

        def q(self, p):
            r = jnp.dot(wall_s[112 * p:112 * (p + 1), :], xn_s[0:D, self.cols], preferred_element_type=f32)
            for gg in range(2):
                pq_s[2 * p + gg] = _features(r[56 * gg:56 * (gg + 1)], T)

        def add(self, v):
            self.acc = (2.0 * x_s[:, self.cols].astype(f32) + v) if self.acc is None else self.acc + v

        def f1(self, c):
            if self.pre_f1:
                self.pre_f1(c)
            hc = jnp.dot(w1T_s[c * FC:(c + 1) * FC, :], xn_s[:, self.cols], preferred_element_type=f32)
            u = hc * (GC + (GC * 0.044715) * (hc * hc))
            self.h[c] = (hc + hc * jnp.tanh(u)).astype(bf16)

        def f2(self, c):
            self.add(jnp.dot(w2T_s[:, c * FC:(c + 1) * FC], self.h.pop(c), preferred_element_type=f32))

        def num(self, g):
            phiq = pq_s[g]
            nT = jnp.dot(kv_s[g], phiq, preferred_element_type=f32)
            rden = pl.reciprocal(nT[56:64] + 1e-6, approx=True)
            self.os.append((nT[0:56].reshape(7, 8, T) * rden[None]).reshape(56, T))

        def wo(self):
            if self.pre_wo:
                self.pre_wo()
            oT = jnp.concatenate(self.os + [(_iota((64, T), 0) == 0).astype(f32)], axis=0).astype(bf16)
            self.add(jnp.dot(woT_s[...], oT, preferred_element_type=f32))

        def store(self):
            o_ref[...] = (0.5 * self.acc).astype(bf16)

    @pl.when(step == 0)
    def _step0():
        cps = {}

        def cp(name, src, dst):
            k = len(cps)
            cps[name] = pltpu.make_async_copy(src, dst, sems.at[k])
            cps[name].start()

        def wait(*names):
            for n_ in names:
                cps[n_].wait()

        def tile(j):
            return slice(j * T, (j + 1) * T)

        cp("wphi", wphi_hbm, wphi_s)
        cp("wA", wqkv_hbm.at[:, 384:896], wqkv_s.at[:, 384:896])
        cp("x0", x_hbm.at[:, tile(0)], x_s.at[:, tile(0)])
        cp("wB", wqkv_hbm.at[:, 896:1344], wqkv_s.at[:, 896:1344])
        cp("x1", x_hbm.at[:, tile(1)], x_s.at[:, tile(1)])
        cp("wC", wqkv_hbm.at[:, 0:384], wqkv_s.at[:, 0:384])
        cp("x2", x_hbm.at[:, tile(2)], x_s.at[:, tile(2)])
        cp("x3", x_hbm.at[:, tile(3)], x_s.at[:, tile(3)])
        cp("b1", b1_hbm, b1_s)
        cp("b2", b2_hbm, b2_s)
        cp("w1", w1_hbm, w1_s)
        cp("w2", w2T_hbm, w2T_s)
        cp("wo", wo_hbm, wo_s)

        kwin = [(0, 256), (128, 384), (256, 512), (384, 512)]
        qwin = [(0, 128), (0, 256), (128, 384), (256, 512)]
        _, rr2 = _divmod_const(_iota((112, 128), 0), 56)
        rt = ((rr2 >> 1) == _iota((112, 128), 1)).astype(bf16)

        def mask(G, lo, hi, shift):
            n = hi - lo
            rg, rr = _divmod_const(_iota((112, n), 0), 56)
            rh = 4 * G + rg * 2 + (rr & 1)
            ch, _ = _divmod_const(jnp.maximum(_iota((112, n), 1) + (lo - shift), 0), DH)
            return rh == ch

        kmask = [mask(G, *kwin[G], 64) for G in range(4)]
        tmpa_s[0, 0:D, :] = jnp.zeros((D, 128), f32)
        wfl_s[0:64, :] = jnp.zeros((64, 128), f32)
        wfl_s[512:576, :] = jnp.zeros((64, 128), f32)

        wait("wphi")
        tmpa_s[0, 0:D, 0:DH] = wphi_s[...].astype(f32)
        for h in range(H):
            wfl_s[64 + h * DH:64 + (h + 1) * DH, :] = tmpa_s[0, pl.ds(h, DH, stride=H), :]
        wfl = wfl_s[...].astype(bf16)
        bd_k = [jnp.where(kmask[G], lax.dot_general(rt, wfl[kwin[G][0]:kwin[G][1]], NT, preferred_element_type=f32), 0.0).astype(bf16)
                for G in range(4)]

        def chunk(j, n):
            return slice(j * T + n * LNC, j * T + (n + 1) * LNC)

        ln_done = set()

        def ln(j, n):
            if (j, n) in ln_done:
                return
            ln_done.add((j, n))
            sl = chunk(j, n)
            x = x_s[:, sl].astype(f32)
            mu = jnp.mean(x, axis=0, keepdims=True)
            xc = x - mu
            var = jnp.mean(xc * xc, axis=0, keepdims=True)
            xn_s[0:D, sl] = (xc * lax.rsqrt(var + 1e-5)).astype(bf16)
            xn_s[D:512, sl] = (_iota((64, LNC), 0) == 0).astype(bf16)

        bd_q = [jnp.where(mask(G, *qwin[G], 0), lax.dot_general(rt, wfl[64 + qwin[G][0]:64 + qwin[G][1]], NT, preferred_element_type=f32), 0.0).astype(bf16)
                for G in range(4)]

        wait("wA")
        for G in range(4):
            lo, hi = kwin[G]
            wk_ = lax.dot_general(
                bd_k[G], wqkv_s[:, 384 + lo:384 + hi], NT, preferred_element_type=f32)
            wall_s[D + 112 * G:D + 112 * (G + 1), :] = (wk_ * LOG2E).astype(bf16)

        def wv_prep():
            wvT = jnp.concatenate([wqkv_s[:, 896:1344].astype(f32), jnp.zeros((64, D), f32)], axis=0).T
            for c in range(4):
                for h in range(H):
                    tmpa_s[c, pl.ds(56 * (h // 2) + (h % 2), DH, stride=2), :] = wvT[h * DH:(h + 1) * DH, 128 * c:128 * (c + 1)]
            wall_s[2 * D:3 * D, :] = jnp.concatenate([tmpa_s[c, 0:D, :] for c in range(4)], axis=1)[:, 0:D].astype(bf16)

        def wq_prep(G):
            lo, hi = qwin[G]
            bd = bd_q[G]
            wall_s[112 * G:112 * (G + 1), :] = (lax.dot_general(
                bd, wqkv_s[:, lo:hi], NT, preferred_element_type=f32) * LOG2E).astype(bf16)

        ones8 = jnp.ones((8, LNC), f32)

        def st_v(j, n, r):
            for g in range(8):
                vas[j][g, :, n * LNC:(n + 1) * LNC] = jnp.concatenate([r[56 * g:56 * (g + 1)], ones8], axis=0).astype(bf16)

        def st_k(j, n, r):
            for g in range(8):
                pks[j][g, :, n * LNC:(n + 1) * LNC] = _features(r[56 * g:56 * (g + 1)], LNC)

        def mm_k(j, n):
            ln(j, n)
            st_k(j, n, jnp.dot(wall_s[D:2 * D, :], xn_s[0:D, chunk(j, n)], preferred_element_type=f32))

        def mm_v(j, n):
            st_v(j, n, jnp.dot(wall_s[2 * D:3 * D, :], xn_s[0:D, chunk(j, n)], preferred_element_type=f32))

        def mm_kv(j, n):
            ln(j, n)
            r = jnp.dot(wall_s[D:3 * D, :], xn_s[0:D, chunk(j, n)], preferred_element_type=f32)
            st_k(j, n, r[0:D])
            st_v(j, n, r[D:2 * D])

        def mm_q0(n):
            r = jnp.dot(wall_s[0:D, :], xn_s[0:D, chunk(0, n)], preferred_element_type=f32)
            for g in range(8):
                pq_s[g, :, n * LNC:(n + 1) * LNC] = _features(r[56 * g:56 * (g + 1)], LNC)

        kv_acc = [None] * 8
        keep = (_iota((64, 112), 0) & 1) == (_iota((64, 112), 1) & 1)

        def kvacc(j, g):
            phik = pks[j][g]
            r = lax.dot_general(vas[j][g], phik, NT, preferred_element_type=f32)
            kv_acc[g] = r if kv_acc[g] is None else kv_acc[g] + r
            if j == NTL - 1:
                kv_s[g] = jnp.where(keep, kv_acc[g], 0.0).astype(bf16)

        tr_done = set()

        def w1_tr(c):
            if c in tr_done:
                return
            tr_done.add(c)
            cs = slice(c * 256, (c + 1) * 256)
            b1blk = jnp.where(_iota((64, 256), 0) == 0, b1_s[...].astype(f32).reshape(1, F)[:, cs], 0.0).astype(bf16)
            w1T_s[cs, :] = jnp.concatenate([w1_s[:, cs], b1blk], axis=0).T

        def wo_prep():
            wo = jnp.concatenate([wo_s[...].astype(f32), jnp.zeros((D, 64), f32)], axis=1)
            b2blk = jnp.where(_iota((64, D), 0) == 0, b2_s[...].astype(f32).reshape(1, D), 0.0)
            b2blk = jnp.concatenate([b2blk, jnp.zeros((64, 64), f32)], axis=1)
            for c in range(4):
                for h in range(H):
                    tmpb_s[c, pl.ds(56 * (h // 2) + (h % 2), DH, stride=2), :] = wo[h * DH:(h + 1) * DH, 128 * c:128 * (c + 1)]
                tmpb_s[c, D:512, :] = b2blk[:, 128 * c:128 * (c + 1)]
                n = 128 if c < 3 else 64
                woT_s[128 * c:128 * c + n, :] = (tmpb_s[c].T[0:n] * 2.0).astype(bf16)

        t0 = Tile(tile(0), pre_f1=w1_tr, pre_wo=wo_prep)
        for tok in SEQ0.split():
            op, ar = tok[0], [int(ch) for ch in tok[1:] if ch.isdigit()]
            if op == 'K': mm_k(*ar)
            elif op == 'V': mm_v(*ar)
            elif op == 'W': mm_kv(*ar)
            elif op == 'Q': mm_q0(*ar)
            elif op == 'k': kvacc(*ar)
            elif op == 'a': t0.f1(*ar)
            elif op == 'b': t0.f2(*ar)
            elif op == 'n': t0.num(*ar)
            elif op == 'w': t0.wo()
            elif op == 'L': ln(*ar)
            elif op == 'T': w1_tr(*ar)
            elif op == 'P': wq_prep(*ar)
            elif op == 'v': wv_prep()
            elif op == '|': wait(*tok[1:].split(','))
            else: raise ValueError(tok)
        t0.store()

    @pl.when(step > 0)
    def _stepn():
        col0 = pl.multiple_of(step * T, T)
        tt = Tile(pl.ds(col0, T))
        for tok in SEQN.split():
            op, ar = tok[0], [int(ch) for ch in tok[1:] if ch.isdigit()]
            if op == 'q': tt.q(*ar)
            elif op == 'a': tt.f1(*ar)
            elif op == 'b': tt.f2(*ar)
            elif op == 'n': tt.num(*ar)
            elif op == 'w': tt.wo()
            else: raise ValueError(tok)
        tt.store()


@jax.jit
def pallas_parallel_sum__linear_kernel_hedgehog__dense_activation_gelu__prompt_kernel(
    A_x, A_wqkv, A_w_phi, A_wo, B_x, B_w1, B_b1, B_w2, B_b2):
    xT = A_x.reshape(S, D).T
    wphi2 = A_w_phi.transpose(1, 0, 2).reshape(D, DH)
    w2T = B_w2.T
    hbm = pl.BlockSpec(memory_space=pl.ANY)
    out = pl.pallas_call(
        _kernel,
        grid=(NTL,),
        in_specs=[hbm] * 8,
        out_specs=pl.BlockSpec((D, T), lambda s: (0, s)),
        out_shape=jax.ShapeDtypeStruct((D, S), bf16),
        scratch_shapes=[
            pltpu.VMEM((D, S), bf16),
            pltpu.VMEM((D, 3 * D), bf16),
            pltpu.VMEM((D, DH), bf16),
            pltpu.VMEM((D, D), bf16),
            pltpu.VMEM((D, F), bf16),
            pltpu.VMEM((F,), bf16),
            pltpu.VMEM((D, F), bf16),
            pltpu.VMEM((D,), bf16),
            pltpu.SemaphoreType.DMA((24,)),
            pltpu.VMEM((512, S), bf16),
            pltpu.VMEM((8, 112, T), bf16),
            pltpu.VMEM((8, 112, T), bf16), pltpu.VMEM((8, 112, T), bf16), pltpu.VMEM((8, 112, T), bf16), pltpu.VMEM((8, 112, T), bf16),
            pltpu.VMEM((8, 64, T), bf16), pltpu.VMEM((8, 64, T), bf16), pltpu.VMEM((8, 64, T), bf16), pltpu.VMEM((8, 64, T), bf16),
            pltpu.VMEM((3 * D, D), bf16),
            pltpu.VMEM((D, 512), bf16),
            pltpu.VMEM((F, 512), bf16),
            pltpu.VMEM((8, 64, 112), bf16),
            pltpu.VMEM((4, D, 128), f32),
            pltpu.VMEM((4, 512, 128), f32),
            pltpu.VMEM((576, 128), f32),
        ],
        compiler_params=pltpu.CompilerParams(
            dimension_semantics=("arbitrary",),
            vmem_limit_bytes=100 * 1024 * 1024),
    )(xT, A_wqkv, wphi2, A_wo, B_w1, B_b1, w2T, B_b2)
    return out.T.reshape(1, S, D)
```

```python
import functools
import jax
import jax.numpy as jnp
from jax import lax
from jax.experimental import pallas as pl
from jax.experimental.pallas import tpu as pltpu

S, D, H, DH, F = 2048, 448, 16, 28, 1792
NT = (((1,), (1,)), ((), ()))
T = 512
TG = 768
NG = (S - T) // TG
NTL = S // T
FC = 256
NC = F // FC
LNC = 128
SEQ0 = (
    "|x0 K00 K01 K02 K03 |wB,wC,x1 v P0 P1 P2 P3 Q0 Q1 Q2 Q3 V00 "
    "V01 V02 V03 K10 V10 K11 V11 K12 K13 V12 |x2,x3,b1,b2,w1 V13 K20 V20 k00 k01 "
    "k02 k03 k04 k05 k06 k07 K21 V21 K22 k10 k11 V22 k12 k13 K23 k14 "
    "k15 V23 k16 k17 a0 K30 V30 a1 K31 k20 k21 V31 |w2,wo k22 k23 b0 "
    "K32 k24 k25 V32 k26 k27 a2 K33 V33 b1 k30 k31 k32 k33 k34 k35 "
    "k36 k37 a3 b2 n0 n1 a4 b3 n2 n3 n4 a5 n5 b4 n6 n7 "
    "a6 w B "
)
SEQN = "q0 q1 q2 q3 a0 a1 b0 n0 n1 a2 b1 n2 n3 a3 b2 n4 n5 a4 b3 n6 n7 a5 b4 w a6 B"
f32 = jnp.float32
LOG2E = 1.4426950408889634
GC = 0.7978845608028654
bf16 = jnp.bfloat16
P = functools.partial
u32 = jnp.uint32


def _pk(v):
    return pltpu.bitcast(v, u32)


def _up(v):
    return pltpu.bitcast(v, bf16)


def _iota(shape, dim):
    return lax.broadcasted_iota(jnp.int32, shape, dim)


def _divmod_const(i, n):
    q = jnp.floor((i.astype(f32) + 0.5) * (1.0 / n)).astype(jnp.int32)
    return q, i - q * n


def _fold(x, op):
    x = op(x, pltpu.roll(x, 4, 0))
    return op(x, pltpu.roll(x, 2, 0))


def _features(pg, t):
    p = pg.reshape(7, 8, t)
    mx = _fold(jnp.max(p, axis=0), jnp.maximum)
    mn = _fold(jnp.min(p, axis=0), jnp.minimum)

    def half(e):
        s = _fold(jnp.sum(e, axis=0), jnp.add)
        return (e * pl.reciprocal(s, approx=True)[None]).reshape(56, t)

    pos = half(jnp.exp2(p - mx[None]))
    neg = half(jnp.exp2(mn[None] - p))
    return jnp.concatenate([pos, neg], axis=0).astype(bf16)


def _kernel(x_hbm, wqkv_hbm, wphi_hbm, wo_hbm, w1_hbm, b1_hbm, w2T_hbm, b2_hbm, o_hbm,
            x_s, wqkv_s, wphi_s, wo_s, w1_s, b1_s, w2T_s, b2_s, sems,
            xn_s, pq_s, pk0, pk1, pk2, pk3, va0, va1, va2, va3, wall_s, woT_s, w1T_s, kv_s, tmpa_s, tmpb_s, wfl_s, out_s):
    step = pl.program_id(0)
    pks = [pk0, pk1, pk2, pk3]
    vas = [va0, va1, va2, va3]

    class Tile:
        def __init__(self, cols, col0, t, pre_f1=None, pre_wo=None):
            self.cols = cols
            self.t = t
            self.col0 = col0
            self.h = {}
            self.acc = None
            self.os = []
            self.pre_f1 = pre_f1
            self.pre_wo = pre_wo

        def q(self, p):
            r = jnp.dot(_up(wall_s[56 * p:56 * (p + 1), :]), _up(xn_s[0:D // 2, self.cols]), preferred_element_type=f32)
            for gg in range(2):
                pq_s[2 * p + gg, :, 0:self.t] = _pk(_features(r[56 * gg:56 * (gg + 1)], self.t))

        def add(self, v):
            self.acc = (2.0 * x_s[:, self.cols].astype(f32) + v) if self.acc is None else self.acc + v

        def f1(self, c):
            if self.pre_f1:
                self.pre_f1(c)
            hc = jnp.dot(_up(w1T_s[c * FC // 2:(c + 1) * FC // 2, :]), _up(xn_s[:, self.cols]), preferred_element_type=f32)
            u = hc * (GC + (GC * 0.044715) * (hc * hc))
            self.h[c] = (hc + hc * jnp.tanh(u)).astype(bf16)

        def f2(self, c):
            self.add(jnp.dot(w2T_s[:, c * FC:(c + 1) * FC], self.h.pop(c), preferred_element_type=f32))

        def num(self, g):
            phiq = _up(pq_s[g, :, 0:self.t])
            nT = jnp.dot(_up(kv_s[g]), phiq, preferred_element_type=f32)
            rden = pl.reciprocal(nT[56:64] + 1e-6, approx=True)
            self.os.append((nT[0:56].reshape(7, 8, self.t) * rden[None]).reshape(56, self.t))

        def wo(self):
            if self.pre_wo:
                self.pre_wo()
            oT = jnp.concatenate(self.os + [(_iota((64, self.t), 0) == 0).astype(f32)], axis=0).astype(bf16)
            self.add(jnp.dot(_up(woT_s[...]), oT, preferred_element_type=f32))

        def out_copy(self, n):
            c0 = self.col0 + n * 128
            if not isinstance(c0, int):
                c0 = pl.multiple_of(c0, 128)
            return pltpu.make_async_copy(out_s.at[:, pl.ds(c0, 128)], o_hbm.at[:, pl.ds(c0, 128)], sems.at[0])

        def final(self):
            hh = jnp.concatenate([self.h.pop(NC - 2), self.h.pop(NC - 1)], axis=0)
            for n in range(self.t // 128):
                cs = slice(n * 128, (n + 1) * 128)
                r = self.acc[:, cs] + jnp.dot(w2T_s[:, (NC - 2) * FC:NC * FC], hh[:, cs], preferred_element_type=f32)
                c0 = self.col0 + n * 128
                if not isinstance(c0, int):
                    c0 = pl.multiple_of(c0, 128)
                out_s[:, pl.ds(c0, 128)] = (0.5 * r).astype(bf16)
                self.out_copy(n).start()

    @pl.when(step == 0)
    def _step0():
        cps = {}

        grp = {"wphi": 0, "wA": 1, "x0": 2, "wB": 3, "wC": 3, "x1": 3, "x2": 4, "x3": 4, "b1": 4, "b2": 4, "w1": 4, "w2": 5, "wo": 5}

        def cp(name, src, dst):
            cps[name] = pltpu.make_async_copy(src, dst, sems.at[grp[name]])
            cps[name].start()

        def wait(*names):
            for n_ in names:
                cps[n_].wait()

        def tile(j):
            return slice(j * T, (j + 1) * T)

        cp("wphi", wphi_hbm, wphi_s)
        cp("wA", wqkv_hbm.at[:, 384:896], wqkv_s.at[:, 384:896])
        cp("x0", x_hbm.at[:, tile(0)], x_s.at[:, tile(0)])
        cp("wB", wqkv_hbm.at[:, 896:1344], wqkv_s.at[:, 896:1344])
        cp("x1", x_hbm.at[:, tile(1)], x_s.at[:, tile(1)])
        cp("wC", wqkv_hbm.at[:, 0:384], wqkv_s.at[:, 0:384])
        cp("x2", x_hbm.at[:, tile(2)], x_s.at[:, tile(2)])
        cp("x3", x_hbm.at[:, tile(3)], x_s.at[:, tile(3)])
        cp("b1", b1_hbm, b1_s)
        cp("b2", b2_hbm, b2_s)
        cp("w1", w1_hbm, w1_s)
        cp("w2", w2T_hbm, w2T_s)
        cp("wo", wo_hbm, wo_s)

        kwin = [(0, 256), (128, 384), (256, 512), (384, 512)]
        qwin = [(0, 128), (0, 256), (128, 384), (256, 512)]
        _, rr2 = _divmod_const(_iota((112, 128), 0), 56)
        rt = ((rr2 >> 1) == _iota((112, 128), 1)).astype(bf16)

        def mask(G, lo, hi, shift):
            n = hi - lo
            rg, rr = _divmod_const(_iota((112, n), 0), 56)
            rh = 4 * G + rg * 2 + (rr & 1)
            ch, _ = _divmod_const(jnp.maximum(_iota((112, n), 1) + (lo - shift), 0), DH)
            return rh == ch

        kmask = [mask(G, *kwin[G], 64) for G in range(4)]
        tmpa_s[0, 0:D, :] = jnp.zeros((D, 128), f32)
        wfl_s[0:64, :] = jnp.zeros((64, 128), f32)
        wfl_s[512:576, :] = jnp.zeros((64, 128), f32)

        wait("wphi")
        tmpa_s[0, 0:D, 0:DH] = wphi_s[...].astype(f32)
        for h in range(H):
            wfl_s[64 + h * DH:64 + (h + 1) * DH, :] = tmpa_s[0, pl.ds(h, DH, stride=H), :]
        wfl = wfl_s[...].astype(bf16)
        bd_k = [jnp.where(kmask[G], lax.dot_general(rt, wfl[kwin[G][0]:kwin[G][1]], NT, preferred_element_type=f32), 0.0).astype(bf16)
                for G in range(4)]

        def chunk(j, n):
            return slice(j * T + n * LNC, j * T + (n + 1) * LNC)

        ln_done = set()

        def ln(j, n):
            if (j, n) in ln_done:
                return
            ln_done.add((j, n))
            sl = chunk(j, n)
            x = x_s[:, sl].astype(f32)
            mu = jnp.mean(x, axis=0, keepdims=True)
            xc = x - mu
            var = jnp.mean(xc * xc, axis=0, keepdims=True)
            xn_s[0:D // 2, sl] = _pk((xc * lax.rsqrt(var + 1e-5)).astype(bf16))
            xn_s[D // 2:256, sl] = _pk((_iota((64, LNC), 0) == 0).astype(bf16))

        bd_q = [jnp.where(mask(G, *qwin[G], 0), lax.dot_general(rt, wfl[64 + qwin[G][0]:64 + qwin[G][1]], NT, preferred_element_type=f32), 0.0).astype(bf16)
                for G in range(4)]

        wait("wA")
        for G in range(4):
            lo, hi = kwin[G]
            wk_ = lax.dot_general(
                bd_k[G], wqkv_s[:, 384 + lo:384 + hi], NT, preferred_element_type=f32)
            wall_s[224 + 56 * G:224 + 56 * (G + 1), :] = _pk((wk_ * LOG2E).astype(bf16))

        def wv_prep():
            wvT = jnp.concatenate([wqkv_s[:, 896:1344].astype(f32), jnp.zeros((64, D), f32)], axis=0).T
            for c in range(4):
                for h in range(H):
                    tmpa_s[c, pl.ds(56 * (h // 2) + (h % 2), DH, stride=2), :] = wvT[h * DH:(h + 1) * DH, 128 * c:128 * (c + 1)]
            wall_s[D:D + 224, :] = _pk(jnp.concatenate([tmpa_s[c, 0:D, :] for c in range(4)], axis=1)[:, 0:D].astype(bf16))

        def wq_prep(G):
            lo, hi = qwin[G]
            bd = bd_q[G]
            wall_s[56 * G:56 * (G + 1), :] = _pk((lax.dot_general(
                bd, wqkv_s[:, lo:hi], NT, preferred_element_type=f32) * LOG2E).astype(bf16))

        ones8 = jnp.ones((8, LNC), f32)

        def st_v(j, n, r):
            for g in range(8):
                vas[j][g, :, n * LNC:(n + 1) * LNC] = _pk(jnp.concatenate([r[56 * g:56 * (g + 1)], ones8], axis=0).astype(bf16))

        def st_k(j, n, r):
            for g in range(8):
                pks[j][g, :, n * LNC:(n + 1) * LNC] = _pk(_features(r[56 * g:56 * (g + 1)], LNC))

        def mm_k(j, n):
            ln(j, n)
            st_k(j, n, jnp.dot(_up(wall_s[224:D, :]), _up(xn_s[0:D // 2, chunk(j, n)]), preferred_element_type=f32))

        def mm_v(j, n):
            st_v(j, n, jnp.dot(_up(wall_s[D:D + 224, :]), _up(xn_s[0:D // 2, chunk(j, n)]), preferred_element_type=f32))

        def mm_kv(j, n):
            ln(j, n)
            r = jnp.dot(_up(wall_s[224:D + 224, :]), _up(xn_s[0:D // 2, chunk(j, n)]), preferred_element_type=f32)
            st_k(j, n, r[0:D])
            st_v(j, n, r[D:2 * D])

        def mm_q0(n):
            r = jnp.dot(_up(wall_s[0:224, :]), _up(xn_s[0:D // 2, chunk(0, n)]), preferred_element_type=f32)
            for g in range(8):
                pq_s[g, :, n * LNC:(n + 1) * LNC] = _pk(_features(r[56 * g:56 * (g + 1)], LNC))

        kv_acc = [None] * 8
        keep = (_iota((64, 112), 0) & 1) == (_iota((64, 112), 1) & 1)

        def kvacc(j, g):
            phik = _up(pks[j][g])
            r = lax.dot_general(_up(vas[j][g]), phik, NT, preferred_element_type=f32)
            kv_acc[g] = r if kv_acc[g] is None else kv_acc[g] + r
            if j == NTL - 1:
                kv_s[g] = _pk(jnp.where(keep, kv_acc[g], 0.0).astype(bf16))

        tr_done = set()

        def w1_tr(c):
            if c in tr_done:
                return
            tr_done.add(c)
            cs = slice(c * 256, (c + 1) * 256)
            b1blk = jnp.where(_iota((64, 256), 0) == 0, b1_s[...].astype(f32).reshape(1, F)[:, cs], 0.0).astype(bf16)
            w1T_s[c * 128:(c + 1) * 128, :] = _pk(jnp.concatenate([w1_s[:, cs], b1blk], axis=0).T)

        def wo_prep():
            wo = jnp.concatenate([wo_s[...].astype(f32), jnp.zeros((D, 64), f32)], axis=1)
            b2blk = jnp.where(_iota((64, D), 0) == 0, b2_s[...].astype(f32).reshape(1, D), 0.0)
            b2blk = jnp.concatenate([b2blk, jnp.zeros((64, 64), f32)], axis=1)
            for c in range(4):
                for h in range(H):
                    tmpb_s[c, pl.ds(56 * (h // 2) + (h % 2), DH, stride=2), :] = wo[h * DH:(h + 1) * DH, 128 * c:128 * (c + 1)]
                tmpb_s[c, D:512, :] = b2blk[:, 128 * c:128 * (c + 1)]
                n = 128 if c < 3 else 64
                woT_s[64 * c:64 * c + n // 2, :] = _pk((tmpb_s[c].T[0:n] * 2.0).astype(bf16))

        t0 = Tile(tile(0), 0, T, pre_f1=w1_tr, pre_wo=wo_prep)
        for tok in SEQ0.split():
            op, ar = tok[0], [int(ch) for ch in tok[1:] if ch.isdigit()]
            if op == 'K': mm_k(*ar)
            elif op == 'V': mm_v(*ar)
            elif op == 'W': mm_kv(*ar)
            elif op == 'Q': mm_q0(*ar)
            elif op == 'k': kvacc(*ar)
            elif op == 'a': t0.f1(*ar)
            elif op == 'b': t0.f2(*ar)
            elif op == 'n': t0.num(*ar)
            elif op == 'w': t0.wo()
            elif op == 'B': t0.final()
            elif op == 'L': ln(*ar)
            elif op == 'T': w1_tr(*ar)
            elif op == 'P': wq_prep(*ar)
            elif op == 'v': wv_prep()
            elif op == '|': wait(*tok[1:].split(','))
            else: raise ValueError(tok)

    @pl.when(step > 0)
    def _stepn():
        col0 = pl.multiple_of(T + (step - 1) * TG, 128)
        tt = Tile(pl.ds(col0, TG), col0, TG)
        for tok in SEQN.split():
            op, ar = tok[0], [int(ch) for ch in tok[1:] if ch.isdigit()]
            if op == 'q': tt.q(*ar)
            elif op == 'a': tt.f1(*ar)
            elif op == 'b': tt.f2(*ar)
            elif op == 'n': tt.num(*ar)
            elif op == 'w': tt.wo()
            elif op == 'B': tt.final()
            else: raise ValueError(tok)

    @pl.when(step == NG)
    def _drain():
        for k in range(4 * NTL):
            pltpu.make_async_copy(out_s.at[:, k * 128:(k + 1) * 128], o_hbm.at[:, k * 128:(k + 1) * 128], sems.at[0]).wait()


@jax.jit
def pallas_parallel_sum__linear_kernel_hedgehog__dense_activation_gelu__prompt_kernel(
    A_x, A_wqkv, A_w_phi, A_wo, B_x, B_w1, B_b1, B_w2, B_b2):
    xT = A_x.reshape(S, D).T
    wphi2 = A_w_phi.transpose(1, 0, 2).reshape(D, DH)
    w2T = B_w2.T
    hbm = pl.BlockSpec(memory_space=pl.ANY)
    out = pl.pallas_call(
        _kernel,
        grid=(1 + NG,),
        in_specs=[hbm] * 8,
        out_specs=hbm,
        out_shape=jax.ShapeDtypeStruct((D, S), bf16),
        scratch_shapes=[
            pltpu.VMEM((D, S), bf16),
            pltpu.VMEM((D, 3 * D), bf16),
            pltpu.VMEM((D, DH), bf16),
            pltpu.VMEM((D, D), bf16),
            pltpu.VMEM((D, F), bf16),
            pltpu.VMEM((F,), bf16),
            pltpu.VMEM((D, F), bf16),
            pltpu.VMEM((D,), bf16),
            pltpu.SemaphoreType.DMA((6,)),
            pltpu.VMEM((256, S), u32),
            pltpu.VMEM((8, 56, TG), u32),
            pltpu.VMEM((8, 56, T), u32), pltpu.VMEM((8, 56, T), u32), pltpu.VMEM((8, 56, T), u32), pltpu.VMEM((8, 56, T), u32),
            pltpu.VMEM((8, 32, T), u32), pltpu.VMEM((8, 32, T), u32), pltpu.VMEM((8, 32, T), u32), pltpu.VMEM((8, 32, T), u32),
            pltpu.VMEM((3 * D // 2, D), u32),
            pltpu.VMEM((D // 2, 512), u32),
            pltpu.VMEM((F // 2, 512), u32),
            pltpu.VMEM((8, 32, 112), u32),
            pltpu.VMEM((4, D, 128), f32),
            pltpu.VMEM((4, 512, 128), f32),
            pltpu.VMEM((576, 128), f32),
            pltpu.VMEM((D, S), bf16),
        ],
        compiler_params=pltpu.CompilerParams(
            dimension_semantics=("arbitrary",),
            vmem_limit_bytes=100 * 1024 * 1024),
    )(xT, A_wqkv, wphi2, A_wo, B_w1, B_b1, w2T, B_b2)
    return out.T.reshape(1, S, D)
```

```python
import jax
import jax.numpy as jnp
from jax import lax
from jax.experimental import pallas as pl
from jax.experimental.pallas import tpu as pltpu

S, D, H, DH, F = 2048, 448, 16, 28, 1792
NT = (((1,), (1,)), ((), ()))
T = 512
TG = 768
NG = (S - T) // TG
NTL = S // T
FC = 256
NC = F // FC
LNC = 128
SEQ0 = (
    "|x0 K00 K01 K02 K03 |wB,wC v P0 P1 P2 P3 Q0 Q1 Q2 Q3 V00 "
    "V01 V02 |x1,x2,x3 V03 K10 V10 K11 V11 K12 V12 K13 V13 K20 V20 k00 k01 "
    "k02 k03 k04 k05 k06 k07 K21 K22 V21 |b1,b2,w1,w2,wo V22 k10 k11 k12 k13 K23 "
    "k14 k15 V23 k16 k17 a0 K30 V30 a1 K31 k20 k21 V31 k22 k23 b0 "
    "K32 k24 k25 V32 k26 k27 a2 K33 V33 b1 k30 k31 k32 k33 k34 k35 "
    "k36 k37 a3 b2 n0 n1 a4 b3 n2 n3 n4 a5 n5 b4 n6 n7 "
    "a6 w B "
)
SEQN = "q0 q1 q2 q3 a0 a1 b0 n0 n1 a2 b1 n2 n3 a3 b2 n4 n5 a4 b3 n6 n7 a5 b4 w a6 B"
LOG2E = 1.4426950408889634
GC = 0.7978845608028654
f32 = jnp.float32
bf16 = jnp.bfloat16
u32 = jnp.uint32


def _pk(v):
    return pltpu.bitcast(v, u32)


def _up(v):
    return pltpu.bitcast(v, bf16)


def _iota(shape, dim):
    return lax.broadcasted_iota(jnp.int32, shape, dim)


def _divmod_const(i, n):
    q = jnp.floor((i.astype(f32) + 0.5) * (1.0 / n)).astype(jnp.int32)
    return q, i - q * n


def _fold(x, op):
    x = op(x, pltpu.roll(x, 4, 0))
    return op(x, pltpu.roll(x, 2, 0))


def _features(pg, t):
    p = pg.reshape(7, 8, t)
    mx = _fold(jnp.max(p, axis=0), jnp.maximum)
    mn = _fold(jnp.min(p, axis=0), jnp.minimum)

    def half(e):
        s = _fold(jnp.sum(e, axis=0), jnp.add)
        return (e * pl.reciprocal(s, approx=True)[None]).reshape(56, t)

    pos = half(jnp.exp2(p - mx[None]))
    neg = half(jnp.exp2(mn[None] - p))
    return jnp.concatenate([pos, neg], axis=0).astype(bf16)


def _kernel(x_hbm, wqkv_hbm, wphi_hbm, wo_hbm, w1_hbm, b1_hbm, w2T_hbm, b2_hbm, o_hbm,
            x_s, wqkv_s, wphi_s, wo_s, w1_s, b1_s, w2T_s, b2_s, sems,
            xn_s, pq_s, pk0, pk1, pk2, pk3, va0, va1, va2, va3, wall_s, woT_s, w1T_s, kv_s,
            tmpa_s, tmpb_s, wfl_s, out_s):
    step = pl.program_id(0)
    pks = [pk0, pk1, pk2, pk3]
    vas = [va0, va1, va2, va3]

    class Tile:
        def __init__(self, cols, col0, t, pre_f1=None, pre_wo=None):
            self.cols, self.col0, self.t = cols, col0, t
            self.h = {}
            self.acc = None
            self.os = []
            self.pre_f1 = pre_f1
            self.pre_wo = pre_wo

        def q(self, p):
            r = jnp.dot(_up(wall_s[56 * p:56 * (p + 1), :]), _up(xn_s[0:D // 2, self.cols]),
                        preferred_element_type=f32)
            for gg in range(2):
                pq_s[2 * p + gg, :, 0:self.t] = _pk(_features(r[56 * gg:56 * (gg + 1)], self.t))

        def add(self, v):
            self.acc = (2.0 * x_s[:, self.cols].astype(f32) + v) if self.acc is None else self.acc + v

        def f1(self, c):
            if self.pre_f1:
                self.pre_f1(c)
            hc = jnp.dot(_up(w1T_s[c * FC // 2:(c + 1) * FC // 2, :]), _up(xn_s[:, self.cols]),
                         preferred_element_type=f32)
            u = hc * (GC + (GC * 0.044715) * (hc * hc))
            self.h[c] = (hc + hc * jnp.tanh(u)).astype(bf16)

        def f2(self, c):
            self.add(jnp.dot(w2T_s[:, c * FC:(c + 1) * FC], self.h.pop(c), preferred_element_type=f32))

        def num(self, g):
            nT = jnp.dot(_up(kv_s[g]), _up(pq_s[g, :, 0:self.t]), preferred_element_type=f32)
            rden = pl.reciprocal(nT[56:64] + 1e-6, approx=True)
            self.os.append((nT[0:56].reshape(7, 8, self.t) * rden[None]).reshape(56, self.t))

        def wo(self):
            if self.pre_wo:
                self.pre_wo()
            one_row = (_iota((64, self.t), 0) == 0).astype(f32)
            oT = jnp.concatenate(self.os + [one_row], axis=0).astype(bf16)
            self.add(jnp.dot(_up(woT_s[...]), oT, preferred_element_type=f32))

        def final(self):
            hh = jnp.concatenate([self.h.pop(NC - 2), self.h.pop(NC - 1)], axis=0)
            for n in range(self.t // 128):
                cs = slice(n * 128, (n + 1) * 128)
                r = self.acc[:, cs] + jnp.dot(w2T_s[:, (NC - 2) * FC:NC * FC], hh[:, cs],
                                              preferred_element_type=f32)
                c0 = self.col0 + n * 128
                if not isinstance(c0, int):
                    c0 = pl.multiple_of(c0, 128)
                out_s[:, pl.ds(c0, 128)] = (0.5 * r).astype(bf16)
                pltpu.make_async_copy(out_s.at[:, pl.ds(c0, 128)], o_hbm.at[:, pl.ds(c0, 128)],
                                      sems.at[0]).start()

        def run(self, op, ar):
            {'q': self.q, 'a': self.f1, 'b': self.f2, 'n': self.num, 'w': self.wo, 'B': self.final}[op](*ar)

    def parse(tok):
        return tok[0], [int(ch) for ch in tok[1:] if ch.isdigit()]

    @pl.when(step == 0)
    def _step0():
        cps = {}
        grp = {"wphi": 0, "wA": 1, "x0": 2, "wB": 3, "wC": 3, "x1": 4, "x2": 4, "x3": 4,
               "b1": 5, "b2": 5, "w1": 5, "w2": 5, "wo": 5}

        def cp(name, src, dst):
            cps[name] = pltpu.make_async_copy(src, dst, sems.at[grp[name]])
            cps[name].start()

        def wait(*names):
            for n_ in names:
                cps[n_].wait()

        def tile(j):
            return slice(j * T, (j + 1) * T)

        def chunk(j, n):
            return slice(j * T + n * LNC, j * T + (n + 1) * LNC)

        cp("wphi", wphi_hbm, wphi_s)
        cp("wA", wqkv_hbm.at[:, 384:896], wqkv_s.at[:, 384:896])
        cp("x0", x_hbm.at[:, tile(0)], x_s.at[:, tile(0)])
        cp("wB", wqkv_hbm.at[:, 896:1344], wqkv_s.at[:, 896:1344])
        cp("wC", wqkv_hbm.at[:, 0:384], wqkv_s.at[:, 0:384])
        for j in range(1, NTL):
            cp(f"x{j}", x_hbm.at[:, tile(j)], x_s.at[:, tile(j)])
        cp("b1", b1_hbm, b1_s)
        cp("b2", b2_hbm, b2_s)
        cp("w1", w1_hbm, w1_s)
        cp("w2", w2T_hbm, w2T_s)
        cp("wo", wo_hbm, wo_s)

        rg, rr = _divmod_const(_iota((112, 128), 0), 56)
        rt = ((rr >> 1) == _iota((112, 128), 1)).astype(bf16)
        rg, rr = _divmod_const(_iota((112, 112), 0), 56)
        ch, _ = _divmod_const(_iota((112, 112), 1), DH)
        same_head = (rg * 2 + (rr & 1)) == ch
        tmpa_s[0, 0:D, :] = jnp.zeros((D, 128), f32)

        wait("wphi")
        tmpa_s[0, 0:D, 0:DH] = wphi_s[...].astype(f32)
        for h in range(H):
            wfl_s[h * DH:(h + 1) * DH, :] = tmpa_s[0, pl.ds(h, DH, stride=H), :]
        bd = [jnp.where(same_head,
                        lax.dot_general(rt, wfl_s[112 * G:112 * (G + 1), :].astype(bf16), NT,
                                        preferred_element_type=f32), 0.0).astype(bf16)
              for G in range(4)]

        def fold_w(G, col0, row0):
            w = lax.dot_general(bd[G], wqkv_s[:, col0 + 112 * G:col0 + 112 * (G + 1)], NT,
                                preferred_element_type=f32)
            wall_s[row0 + 56 * G:row0 + 56 * (G + 1), :] = _pk((w * LOG2E).astype(bf16))

        wait("wA")
        for G in range(4):
            fold_w(G, D, 224)

        def wq_prep(G):
            fold_w(G, 0, 0)

        def perm_row(h):
            return pl.ds(56 * (h // 2) + (h % 2), DH, stride=2)

        def wv_prep():
            wvT = jnp.concatenate([wqkv_s[:, 2 * D:3 * D].astype(f32), jnp.zeros((64, D), f32)], axis=0).T
            for c in range(4):
                for h in range(H):
                    tmpa_s[c, perm_row(h), :] = wvT[h * DH:(h + 1) * DH, 128 * c:128 * (c + 1)]
            wall_s[D:D + 224, :] = _pk(
                jnp.concatenate([tmpa_s[c, 0:D, :] for c in range(4)], axis=1)[:, 0:D].astype(bf16))

        def ln(j, n):
            sl = chunk(j, n)
            x = x_s[:, sl].astype(f32)
            mu = jnp.mean(x, axis=0, keepdims=True)
            xc = x - mu
            var = jnp.mean(xc * xc, axis=0, keepdims=True)
            xn_s[0:D // 2, sl] = _pk((xc * lax.rsqrt(var + 1e-5)).astype(bf16))
            xn_s[D // 2:256, sl] = _pk((_iota((64, LNC), 0) == 0).astype(bf16))

        def proj(row0, j, n):
            return jnp.dot(_up(wall_s[row0:row0 + 224, :]), _up(xn_s[0:D // 2, chunk(j, n)]),
                           preferred_element_type=f32)

        def mm_k(j, n):
            ln(j, n)
            r = proj(224, j, n)
            for g in range(8):
                pks[j][g, :, n * LNC:(n + 1) * LNC] = _pk(_features(r[56 * g:56 * (g + 1)], LNC))

        ones8 = jnp.ones((8, LNC), f32)

        def mm_v(j, n):
            r = proj(D, j, n)
            for g in range(8):
                vas[j][g, :, n * LNC:(n + 1) * LNC] = _pk(
                    jnp.concatenate([r[56 * g:56 * (g + 1)], ones8], axis=0).astype(bf16))

        def mm_q0(n):
            r = proj(0, 0, n)
            for g in range(8):
                pq_s[g, :, n * LNC:(n + 1) * LNC] = _pk(_features(r[56 * g:56 * (g + 1)], LNC))

        kv_acc = [None] * 8
        keep = (_iota((64, 112), 0) & 1) == (_iota((64, 112), 1) & 1)

        def kvacc(j, g):
            r = lax.dot_general(_up(vas[j][g]), _up(pks[j][g]), NT, preferred_element_type=f32)
            kv_acc[g] = r if kv_acc[g] is None else kv_acc[g] + r
            if j == NTL - 1:
                kv_s[g] = _pk(jnp.where(keep, kv_acc[g], 0.0).astype(bf16))

        def w1_tr(c):
            cs = slice(c * FC, (c + 1) * FC)
            b1blk = jnp.where(_iota((64, FC), 0) == 0, b1_s[...].astype(f32).reshape(1, F)[:, cs], 0.0)
            w1T_s[c * FC // 2:(c + 1) * FC // 2, :] = _pk(
                jnp.concatenate([w1_s[:, cs], b1blk.astype(bf16)], axis=0).T)

        def wo_prep():
            wo = jnp.concatenate([wo_s[...].astype(f32), jnp.zeros((D, 64), f32)], axis=1)
            b2blk = jnp.where(_iota((64, D), 0) == 0, b2_s[...].astype(f32).reshape(1, D), 0.0)
            b2blk = jnp.concatenate([b2blk, jnp.zeros((64, 64), f32)], axis=1)
            for c in range(4):
                for h in range(H):
                    tmpb_s[c, perm_row(h), :] = wo[h * DH:(h + 1) * DH, 128 * c:128 * (c + 1)]
                tmpb_s[c, D:512, :] = b2blk[:, 128 * c:128 * (c + 1)]
                n = 128 if c < 3 else 64
                woT_s[64 * c:64 * c + n // 2, :] = _pk((tmpb_s[c].T[0:n] * 2.0).astype(bf16))

        t0 = Tile(tile(0), 0, T, pre_f1=w1_tr, pre_wo=wo_prep)
        ops = {'K': mm_k, 'V': mm_v, 'Q': mm_q0, 'k': kvacc, 'P': wq_prep, 'v': wv_prep}
        for tok in SEQ0.split():
            if tok[0] == '|':
                wait(*tok[1:].split(','))
                continue
            op, ar = parse(tok)
            if op in ops:
                ops[op](*ar)
            else:
                t0.run(op, ar)

    @pl.when(step > 0)
    def _stepn():
        col0 = pl.multiple_of(T + (step - 1) * TG, 128)
        tt = Tile(pl.ds(col0, TG), col0, TG)
        for tok in SEQN.split():
            tt.run(*parse(tok))

    @pl.when(step == NG)
    def _drain():
        for k in range(S // 128):
            pltpu.make_async_copy(out_s.at[:, k * 128:(k + 1) * 128], o_hbm.at[:, k * 128:(k + 1) * 128],
                                  sems.at[0]).wait()


@jax.jit
def pallas_parallel_sum__linear_kernel_hedgehog__dense_activation_gelu__prompt_kernel(
    A_x, A_wqkv, A_w_phi, A_wo, B_x, B_w1, B_b1, B_w2, B_b2):
    xT = A_x.reshape(S, D).T
    wphi2 = A_w_phi.transpose(1, 0, 2).reshape(D, DH)
    w2T = B_w2.T
    hbm = pl.BlockSpec(memory_space=pl.ANY)
    out = pl.pallas_call(
        _kernel,
        grid=(1 + NG,),
        in_specs=[hbm] * 8,
        out_specs=hbm,
        out_shape=jax.ShapeDtypeStruct((D, S), bf16),
        scratch_shapes=[
            pltpu.VMEM((D, S), bf16),
            pltpu.VMEM((D, 3 * D), bf16),
            pltpu.VMEM((D, DH), bf16),
            pltpu.VMEM((D, D), bf16),
            pltpu.VMEM((D, F), bf16),
            pltpu.VMEM((F,), bf16),
            pltpu.VMEM((D, F), bf16),
            pltpu.VMEM((D,), bf16),
            pltpu.SemaphoreType.DMA((6,)),
            pltpu.VMEM((256, S), u32),
            pltpu.VMEM((8, 56, TG), u32),
            pltpu.VMEM((8, 56, T), u32), pltpu.VMEM((8, 56, T), u32),
            pltpu.VMEM((8, 56, T), u32), pltpu.VMEM((8, 56, T), u32),
            pltpu.VMEM((8, 32, T), u32), pltpu.VMEM((8, 32, T), u32),
            pltpu.VMEM((8, 32, T), u32), pltpu.VMEM((8, 32, T), u32),
            pltpu.VMEM((3 * D // 2, D), u32),
            pltpu.VMEM((D // 2, 512), u32),
            pltpu.VMEM((F // 2, 512), u32),
            pltpu.VMEM((8, 32, 112), u32),
            pltpu.VMEM((4, D, 128), f32),
            pltpu.VMEM((4, 512, 128), f32),
            pltpu.VMEM((D, 128), f32),
            pltpu.VMEM((D, S), bf16),
        ],
        compiler_params=pltpu.CompilerParams(
            dimension_semantics=("arbitrary",),
            vmem_limit_bytes=100 * 1024 * 1024),
    )(xT, A_wqkv, wphi2, A_wo, B_w1, B_b1, w2T, B_b2)
    return out.T.reshape(1, S, D)
```
